```python
import os as _os
_os.environ.setdefault("JAX_PLATFORMS", "cpu")
import jax
import jax.numpy as jnp

def _softmax(x, axis=-1):
    return jax.nn.softmax(x, axis=axis)
def _gelu(x):
    return jax.nn.gelu(x, approximate=True)
def _silu(x):
    return jax.nn.silu(x)
def _sigmoid(x):
    return jax.nn.sigmoid(x)
def _layernorm(x, axis=-1, eps=1e-5):
    m = jnp.mean(x, axis=axis, keepdims=True)
    v = jnp.var(x, axis=axis, keepdims=True)
    return (x - m) / jnp.sqrt(v + eps)
def _scatter_add(tgt, idx, src, axis=0):
    return tgt.at[idx].add(src)
def _segment_sum(src, seg, n):
    return jax.ops.segment_sum(src, seg, n)
class _Rng:
    def __init__(self, key):
        self._k = key
    def _next(self):
        self._k, sub = jax.random.split(self._k)
        return sub
    def normal(self, shape):
        return jax.random.normal(self._next(), shape, dtype=jnp.bfloat16)
    def randint(self, lo, hi, shape):
        return jax.random.randint(self._next(), shape, lo, hi, dtype=jnp.int32)
    def uniform(self, shape, lo=0.0, hi=1.0):
        return jax.random.uniform(self._next(), shape, jnp.bfloat16, lo, hi)
    def permutation(self, n):
        return jax.random.permutation(self._next(), n)


kernel_name = 'standalone__gqa_softmax__decode'

def setup_inputs():
    _rng = _Rng(jax.random.key(int.from_bytes(__import__("os").urandom(4), "little")))
    _w = (lambda a: (lambda t: t.astype(jnp.bfloat16) if jnp.issubdtype(t.dtype, jnp.floating) else t)(jnp.asarray(a)))
    B, Hq, Hkv, Sq, Sk, D = 8, 32, 32, 1, 4096, 128
    return {
        "q": _w((lambda *s: _rng.normal(s) * 0.4)(B, Hq, Sq, D)),
        "k": _w((lambda *s: _rng.normal(s) * 0.4)(B, Hkv, Sk, D)),
        "v": _w((lambda *s: _rng.normal(s) * 0.05)(B, Hkv, Sk, D)),
    }

def reference(q, k, v):
    B, Hq, Sq, D = q.shape
    Hkv = k.shape[1]
    rep = Hq // Hkv
    k = jnp.repeat(k, rep, axis=1)
    v = jnp.repeat(v, rep, axis=1)
    scale = D ** -0.5
    scores = jnp.einsum("bhqd,bhkd->bhqk", q, k) * scale
    p = _softmax(scores, axis=-1)
    return jnp.einsum("bhqk,bhkd->bhqd", p, v)
```

```python
import jax
import jax.numpy as jnp
import jax.experimental.pallas as pl
import jax.experimental.pallas.tpu as pltpu

_CHUNK_ROWS = 192
_NBUF = 4


def _chunks(total, rows):
    return [(r0, min(rows, total - r0)) for r0 in range(0, total, rows)]


@jax.jit
def pallas_standalone__gqa_softmax__decode_kernel(
    q: jax.Array,
    k: jax.Array,
    v: jax.Array,
):
    B, Hq, Sq, D = q.shape
    _, Hkv, Sk, _ = k.shape
    assert Sq == 1 and Hq % Hkv == 0
    rep = Hq // Hkv
    n_q = B * Hq
    scale = D ** -0.5
    pieces = _chunks(Sk, _CHUNK_ROWS)

    def kernel(q_ref, k_hbm, v_hbm, o_ref, kbuf, vbuf, q32, o32, sem):
        def start_head(h, slot):
            base = (h // rep) * Sk
            for r0, nr in pieces:
                src = pl.ds(pl.multiple_of(base + r0, 16), nr)
                pltpu.make_async_copy(
                    k_hbm.at[src], kbuf.at[slot, pl.ds(r0, nr)], sem.at[0, slot]
                ).start(priority=0)
                pltpu.make_async_copy(
                    v_hbm.at[src], vbuf.at[slot, pl.ds(r0, nr)], sem.at[1, slot]
                ).start(priority=1)

        for j in range(_NBUF):
            start_head(j, j)
        q32[...] = q_ref[...].astype(jnp.float32)

        def body(h, carry):
            slot = h % _NBUF
            pltpu.make_async_copy(kbuf.at[slot], kbuf.at[slot], sem.at[0, slot]).wait()
            qv = jnp.broadcast_to(q32[pl.ds(h, 1), :], (8, D)).astype(jnp.bfloat16)
            s = jax.lax.dot_general(
                qv, kbuf[slot], (((1,), (1,)), ((), ())),
                preferred_element_type=jnp.float32,
            ) * scale
            m = jnp.max(s, axis=-1, keepdims=True)
            p = jnp.exp(s - m)
            l = jnp.sum(p, axis=-1, keepdims=True)
            pltpu.make_async_copy(vbuf.at[slot], vbuf.at[slot], sem.at[1, slot]).wait()
            o = jnp.dot(
                p.astype(jnp.bfloat16), vbuf[slot], preferred_element_type=jnp.float32
            )
            o32[pl.ds(h, 1), :] = (o / l)[0:1, :]

            @pl.when(h + _NBUF < n_q)
            def _():
                start_head(h + _NBUF, slot)

            return carry

        jax.lax.fori_loop(0, n_q, body, 0)
        o_ref[...] = o32[...].astype(o_ref.dtype)

    out = pl.pallas_call(
        kernel,
        in_specs=[
            pl.BlockSpec(memory_space=pltpu.VMEM),
            pl.BlockSpec(memory_space=pl.ANY),
            pl.BlockSpec(memory_space=pl.ANY),
        ],
        out_specs=pl.BlockSpec(memory_space=pltpu.VMEM),
        out_shape=jax.ShapeDtypeStruct((n_q, D), q.dtype),
        scratch_shapes=[
            pltpu.VMEM((_NBUF, Sk, D), k.dtype),
            pltpu.VMEM((_NBUF, Sk, D), v.dtype),
            pltpu.VMEM((n_q, D), jnp.float32),
            pltpu.VMEM((n_q, D), jnp.float32),
            pltpu.SemaphoreType.DMA((2, _NBUF)),
        ],
        compiler_params=pltpu.CompilerParams(vmem_limit_bytes=32 * 1024 * 1024),
    )(q.reshape(n_q, D), k.reshape(B * Hkv * Sk, D), v.reshape(B * Hkv * Sk, D))
    return out.reshape(B, Hq, Sq, D)
```

```python
import jax
import jax.numpy as jnp
import jax.experimental.pallas as pl
import jax.experimental.pallas.tpu as pltpu

_NBUF = 4
_CHUNK_ROWS = 192


def _schedule(total, keys_first):
    pieces = [
        (r0, min(_CHUNK_ROWS, total - r0)) for r0 in range(0, total, _CHUNK_ROWS)
    ]
    pairs = [pieces[j:j + 2] for j in range(0, len(pieces), 2)]

    def part(t, groups):
        return [(t, r, n, j) for g in groups for j, (r, n) in enumerate(g)]

    if keys_first:
        return part(0, pairs) + part(1, pairs)
    return [c for g in pairs for c in part(0, [g]) + part(1, [g])]


@jax.jit
def pallas_standalone__gqa_softmax__decode_kernel(
    q: jax.Array,
    k: jax.Array,
    v: jax.Array,
):
    B, Hq, Sq, D = q.shape
    _, Hkv, Sk, _ = k.shape
    assert Sq == 1 and Hq % Hkv == 0 and Sk % 16 == 0
    rep = Hq // Hkv
    n_q = B * Hq
    assert n_q > _NBUF
    scale = D ** -0.5
    steady = _schedule(Sk, False)
    final = _schedule(Sk, True)

    def kernel(q_hbm, k_hbm, v_hbm, o_ref, kbuf, vbuf, qbuf, q32, o32, sem, qsem):
        def start_head(h, slot, schedule):
            base = (h // rep) * Sk
            for t, r0, nr, queue in schedule:
                src, dst = (k_hbm, kbuf) if t == 0 else (v_hbm, vbuf)
                pltpu.make_async_copy(
                    src.at[pl.ds(pl.multiple_of(base + r0, 16), nr)],
                    dst.at[slot, pl.ds(r0, nr)],
                    sem.at[t, slot],
                ).start(priority=queue)

        start_head(0, 0, steady)
        q_copy = pltpu.make_async_copy(q_hbm, qbuf, qsem.at[0])
        q_copy.start()
        for j in range(1, _NBUF):
            start_head(j, j, steady)
        q_copy.wait()
        q32[...] = qbuf[...].astype(jnp.float32)

        def body(h, carry):
            slot = h % _NBUF
            pltpu.make_async_copy(kbuf.at[slot], kbuf.at[slot], sem.at[0, slot]).wait()
            qv = jnp.broadcast_to(q32[pl.ds(h, 1), :], (8, D)).astype(k.dtype)
            s = jax.lax.dot_general(
                qv, kbuf[slot], (((1,), (1,)), ((), ())),
                preferred_element_type=jnp.float32,
            ) * scale
            m = jnp.max(s, axis=-1, keepdims=True)
            p = jnp.exp(s - m)
            l = jnp.sum(p, axis=-1, keepdims=True)
            pltpu.make_async_copy(vbuf.at[slot], vbuf.at[slot], sem.at[1, slot]).wait()
            o = jnp.dot(
                p.astype(v.dtype), vbuf[slot], preferred_element_type=jnp.float32
            )
            o32[pl.ds(h, 1), :] = (o / l)[0:1, :]

            @pl.when(h + _NBUF < n_q - 1)
            def _():
                start_head(h + _NBUF, slot, steady)

            @pl.when(h + _NBUF == n_q - 1)
            def _():
                start_head(h + _NBUF, slot, final)

            return carry

        jax.lax.fori_loop(0, n_q, body, 0)
        o_ref[...] = o32[...].astype(o_ref.dtype)

    out = pl.pallas_call(
        kernel,
        in_specs=[pl.BlockSpec(memory_space=pl.ANY)] * 3,
        out_specs=pl.BlockSpec(memory_space=pltpu.VMEM),
        out_shape=jax.ShapeDtypeStruct((n_q, D), q.dtype),
        scratch_shapes=[
            pltpu.VMEM((_NBUF, Sk, D), k.dtype),
            pltpu.VMEM((_NBUF, Sk, D), v.dtype),
            pltpu.VMEM((n_q, D), q.dtype),
            pltpu.VMEM((n_q, D), jnp.float32),
            pltpu.VMEM((n_q, D), jnp.float32),
            pltpu.SemaphoreType.DMA((2, _NBUF)),
            pltpu.SemaphoreType.DMA((1,)),
        ],
        compiler_params=pltpu.CompilerParams(vmem_limit_bytes=32 * 1024 * 1024),
    )(q.reshape(n_q, D), k.reshape(B * Hkv * Sk, D), v.reshape(B * Hkv * Sk, D))
    return out.reshape(B, Hq, Sq, D)
```
